```python
import os as _os
_os.environ.setdefault('JAX_PLATFORMS', 'cpu')
import jax
import jax.numpy as jnp

def _softmax(x, axis=-1):
    return jax.nn.softmax(x, axis=axis)

def _gelu(x):
    return jax.nn.gelu(x, approximate=True)

def _silu(x):
    return jax.nn.silu(x)

def _sigmoid(x):
    return jax.nn.sigmoid(x)

def _layernorm(x, axis=-1, eps=1e-05):
    m = jnp.mean(x, axis=axis, keepdims=True)
    v = jnp.var(x, axis=axis, keepdims=True)
    return (x - m) / jnp.sqrt(v + eps)

def _scatter_add(tgt, idx, src, axis=0):
    return tgt.at[idx].add(src)

def _segment_sum(src, seg, n):
    return jax.ops.segment_sum(src, seg, n)

class _Rng:

    def __init__(self, key):
        self._k = key

    def _next(self):
        self._k, sub = jax.random.split(self._k)
        return sub

    def normal(self, shape):
        return jax.random.normal(self._next(), shape, dtype=jnp.bfloat16)

    def randint(self, lo, hi, shape):
        return jax.random.randint(self._next(), shape, lo, hi, dtype=jnp.int32)

    def uniform(self, shape, lo=0.0, hi=1.0):
        return jax.random.uniform(self._next(), shape, jnp.bfloat16, lo, hi)

    def permutation(self, n):
        return jax.random.permutation(self._next(), n)
kernel_name = 'concat_heads__ssm_conv_s5__memory_aug_recurrent_mem_tr__prompt'

def setup_inputs():
    _rng = _Rng(jax.random.key(int.from_bytes(__import__("os").urandom(4), "little")))
    _w = lambda a: (lambda t: t.astype(jnp.bfloat16) if jnp.issubdtype(t.dtype, jnp.floating) else t)(jnp.asarray(a))

    def _A_setup():
        B, S, D = (1, 2048, 1024)
        P = D
        Lambda_re = -0.5 * jnp.exp((lambda *s: _rng.normal(s) * 0.8)(P))
        Lambda_im = (lambda *s: _rng.normal(s) * 0.8)(P) * 1.0
        B_re = (lambda *s: _rng.normal(s) * 0.8)(P, D) * D ** (-0.5)
        B_im = (lambda *s: _rng.normal(s) * 0.8)(P, D) * D ** (-0.5)
        C_re = (lambda *s: _rng.normal(s) * 0.8)(D, P) * P ** (-0.5)
        C_im = (lambda *s: _rng.normal(s) * 0.8)(D, P) * P ** (-0.5)
        log_dt = (lambda *s: _rng.normal(s) * 0.8)(P) * 0.3 - 2.0
        Dskip = (lambda *s: _rng.normal(s) * 0.8)(D)
        return {'x': _w((lambda *s: _rng.normal(s) * 0.05)(B, S, D)), 'Lambda_re': _w(Lambda_re), 'Lambda_im': _w(Lambda_im), 'B_re': _w(B_re), 'B_im': _w(B_im), 'C_re': _w(C_re), 'C_im': _w(C_im), 'log_dt': _w(log_dt), 'Dskip': _w(Dskip)}
    _A_in = _A_setup()

    def _B_setup():
        B, S, Dm = (1, 2048, 1024)
        H, Dh = (32, 128)
        M, seg = (8, 32)
        seg = min(seg, S)
        S = S // seg * seg
        return {'x': _w((lambda *s: _rng.normal(s) * 0.05)(B, S, Dm)), 'mem0': _w((lambda *s: _rng.normal(s) * 0.8)(B, M, Dm)), 'Wq': _w((lambda *s: _rng.normal(s) * 1.6)(Dm, H, Dh) * Dm ** (-0.5)), 'Wk': _w((lambda *s: _rng.normal(s) * 1.6)(Dm, H, Dh) * Dm ** (-0.5)), 'Wv': _w((lambda *s: _rng.normal(s) * 0.8)(Dm, H, Dh) * Dm ** (-0.5)), 'Wo': _w((lambda *s: _rng.normal(s) * 0.8)(H, Dh, Dm) * (H * Dh) ** (-0.5)), 'seg_len': seg}
    _B_in = _B_setup()
    return {'A_x': _A_in['x'], 'A_Lambda_re': _A_in['Lambda_re'], 'A_Lambda_im': _A_in['Lambda_im'], 'A_B_re': _A_in['B_re'], 'A_B_im': _A_in['B_im'], 'A_C_re': _A_in['C_re'], 'A_C_im': _A_in['C_im'], 'A_log_dt': _A_in['log_dt'], 'A_Dskip': _A_in['Dskip'], 'B_x': _B_in['x'], 'B_mem0': _B_in['mem0'], 'B_Wq': _B_in['Wq'], 'B_Wk': _B_in['Wk'], 'B_Wv': _B_in['Wv'], 'B_Wo': _B_in['Wo'], 'B_seg_len': _B_in['seg_len']}

def reference(A_x, A_Lambda_re, A_Lambda_im, A_B_re, A_B_im, A_C_re, A_C_im, A_log_dt, A_Dskip, B_x, B_mem0, B_Wq, B_Wk, B_Wv, B_Wo, B_seg_len):

    def _A_ref(x, Lambda_re, Lambda_im, B_re, B_im, C_re, C_im, log_dt, Dskip):
        Bsz, L, H = x.shape
        Lam = Lambda_re + 1j * Lambda_im
        Bmat = B_re + 1j * B_im
        Cmat = C_re + 1j * C_im
        dt = jnp.exp(log_dt)
        Lam_bar = jnp.exp(dt * Lam)
        B_bar = ((Lam_bar - 1.0) / Lam)[:, None] * Bmat
        Bu = jnp.einsum('bld,pd->blp', x + 0j, B_bar)
        h = jnp.zeros_like(Bu[:, 0, :])
        hs = []
        for t in range(L):
            h = Lam_bar[None, :] * h + Bu[:, t, :]
            hs.append(h)
        hseq = jnp.stack(hs, 1)
        y = 2.0 * jnp.einsum('blp,dp->bld', hseq, Cmat).real + x * Dskip[None, None, :]
        return y

    def _B_ref(x, mem0, Wq, Wk, Wv, Wo, seg_len):
        B, S, Dm = x.shape
        H, Dh = (Wq.shape[1], Wq.shape[2])
        M = mem0.shape[1]
        scale = Dh ** (-0.5)
        n_seg = S // seg_len
        L = M + seg_len
        idx = jnp.arange(L)
        mask = (idx[:, None] < M) | (idx[:, None] >= idx[None, :])
        mem = mem0
        outs = []
        for s in range(n_seg):
            xs = x[:, s * seg_len:(s + 1) * seg_len, :].copy()
            h = jnp.concatenate([mem, xs], axis=1)
            q = jnp.einsum('btd,dhe->bhte', h, Wq)
            k = jnp.einsum('btd,dhe->bhte', h, Wk)
            v = jnp.einsum('btd,dhe->bhte', h, Wv)
            scores = jnp.einsum('bhqe,bhke->bhqk', q, k) * scale
            scores = jnp.where(mask[None, None], scores, -1000000000.0)
            p = _softmax(scores, axis=-1)
            o = jnp.einsum('bhqk,bhke->bhqe', p, v)
            o = jnp.einsum('bhte,hed->btd', o, Wo)
            mem = o[:, :M, :].copy()
            outs.append(o[:, M:, :])
        return jnp.concatenate(outs, axis=1)
    a = _A_ref(A_x, A_Lambda_re, A_Lambda_im, A_B_re, A_B_im, A_C_re, A_C_im, A_log_dt, A_Dskip)
    b = _B_ref(B_x, B_mem0, B_Wq, B_Wk, B_Wv, B_Wo, B_seg_len)
    return jnp.concatenate([a, b], axis=-1)
```

```python
import collections
import functools
import itertools

import jax
import jax.numpy as jnp
from jax import lax
import jax.experimental.pallas as pl
import jax.experimental.pallas.tpu as pltpu

F32 = jnp.float32
BF16 = jnp.bfloat16
U32 = jnp.uint32
NT = (((1,), (1,)), ((), ()))
LN = 128
TL = 16
N_MXU = 4
LOG2_E = 1.4426950408889634


class _Scheme:
    def __init__(self, slopes):
        self.t = slopes
        self.n = n = len(slopes)
        self.pairs = list(itertools.combinations(range(n), 2))
        self.slots = 2 * n + 3 * len(self.pairs)

    def R(self, i): return i
    def Q(self, i): return self.n + i
    def S(self, i, j): return 2 * self.n + self.pairs.index((i, j))
    def U(self, i, j): return self.S(i, j) + len(self.pairs)
    def L(self, i, j): return self.U(i, j) + len(self.pairs)

    def pair(self, slot):
        return self.pairs[(slot - 2 * self.n) % len(self.pairs)]

    def left_factors(self, x1, xi):
        @functools.cache
        def factor(slot):
            if slot < 2 * self.n:
                return x1(slot) if slot < self.n else xi(slot - self.n)
            i, j = self.pair(slot)
            d = self.t[i] - self.t[j]
            if slot == self.S(i, j):
                return xi(i) + xi(j)
            if slot == self.U(i, j):
                return factor(self.S(i, j)) + d * x1(i)
            return factor(self.S(i, j)) - d * x1(j)
        return factor

    def combine(self, m, order=None):
        y1, rest = [None] * self.n, [None] * self.n
        for item in order or list(range(self.n)) + self.pairs:
            if isinstance(item, tuple):
                i, j = item
                u, l = m(self.U(i, j)), m(self.L(i, j))
                e = (m(self.S(i, j)) - u - l) * (1.0 / (self.t[i] - self.t[j]))
                _add(y1, i, e)
                _add(y1, j, e, -1)
                _add(rest, j, u)
                _add(rest, i, l)
            else:
                _add(y1, item, m(self.R(item)))
                _add(rest, item, m(self.Q(item)))
        return y1, [rest[j] + self.t[j] * y1[j] for j in range(self.n)]

    def half_slots(self, odd, order, batch):
        slots, pend = [], []
        for item in order:
            if isinstance(item, tuple):
                pend.append(item)
                if len(pend) == batch:
                    slots += [self.S(*p) for p in pend] + [(self.L if odd else self.U)(*p) for p in pend]
                    pend = []
            else:
                slots.append((self.Q if odd else self.R)(item))
        assert not pend
        return slots

    def single_factor(self, odd, a, slot):
        if slot < 2 * self.n:
            return a(slot % self.n)
        i, j = self.pair(slot)
        return a(j) if slot == self.S(i, j) and not odd else a(i) + a(j)

    def single_combine(self, odd, m, order):
        y = [None] * self.n
        for item in order:
            if isinstance(item, tuple):
                i, j = item
                side = m((self.L if odd else self.U)(i, j))
                d = m(self.S(i, j)) - side
                _add(y, i, side if odd else d)
                _add(y, j, d, 1 if odd else -1)
            else:
                _add(y, item, m((self.Q if odd else self.R)(item)))
        return y

    def right_factor_units(self, load, store):
        rows = {}

        def block_row(i):
            rows[i] = load(i)
            for j, (word, _) in enumerate(rows[i]):
                if j != i:
                    store(self.U(i, j) if i < j else self.L(j, i), word)
            store(self.R(i), _round_pack(*(functools.reduce(lax.add, [v[1][h] for v in rows[i]]) for h in range(2))))

        def symmetric(i, j):
            store(self.S(i, j), _round_pack(*map(lax.add, _halves(rows[i][j][0]), rows[j][i][1])))

        def block_column(j):
            wide = lambda i: pltpu.bitcast(rows[i][j][0], BF16).astype(F32)
            total = functools.reduce(lax.sub, [wide(j)] + [wide(i) for i in range(self.n) if i != j])
            store(self.Q(j), pltpu.bitcast(total.astype(BF16), U32))

        units = []
        for j in range(self.n):
            units += [(6 * self.n + 4, functools.partial(block_row, j))]
            units += [(10, functools.partial(symmetric, i, j)) for i in range(j)]
        return units + [(4 * self.n + 3, functools.partial(block_column, j)) for j in range(self.n)]


SSM = _Scheme((-1.375, -0.375, 0.375, 1.375))
ATT = _Scheme((-2.25, -1.125, -0.5625, -0.1875, 0.1875, 0.5625, 1.125, 2.25))


def _add(acc, i, v, sign=1):
    if acc[i] is None:
        acc[i] = v if sign > 0 else -v
    else:
        acc[i] = acc[i] + v if sign > 0 else acc[i] - v


def _cmul(ar, ai, br, bi):
    return ar * br - ai * bi, ar * bi + ai * br


def _halves(word):
    return pltpu.bitcast(word << 16, F32), pltpu.bitcast(word & jnp.uint32(0xFFFF0000), F32)


def _round_pack(lo, hi):
    bits = pltpu.bitcast(jnp.concatenate([lo, hi], axis=1).astype(BF16).astype(F32), U32)
    return (bits[:, :LN] >> 16) | bits[:, LN:]


def _weave(dots, *streams):
    side = []
    for units in streams:
        total, seen = sum(c for c, _ in units), 0
        for c, fn in units:
            side.append(((seen + c / 2) / total, c, fn))
            seen += c
    side.sort(key=lambda v: v[0])
    rate = (sum(c for c, _ in dots) + sum(v[1] for v in side)) / len(dots)
    spent = 0
    for k, (c, fn) in enumerate(dots):
        fn()
        spent += c
        while side and (spent + side[0][1] / 2 <= rate * (k + 1) or k + 1 == len(dots)):
            _, c, fn = side.pop(0)
            fn()
            spent += c


def _start(copies):
    for cp in copies:
        cp.start()


def _wait(copies):
    for cp in copies:
        cp.wait()


def _kernel(
    ax_hbm, lre_hbm, lim_hbm, bre_hbm, bim_hbm, cre_hbm, cim_hbm, ldt_hbm, dsk_hbm,
    bx_hbm, mem0_hbm, wq_hbm, wk_hbm, wv_hbm, wo_hbm,
    out_hbm,
    xp_v, cs_v, wst_v, wqkv_v, wo_v, ga_v, gb_v, prod_v, coef_v, carry_v, o_v, po_v, sems,
    *, seg,
):
    n_blk, _, _, D = ax_hbm.shape
    tb, hb = 8 * TL, 4 * TL
    S = n_blk * tb
    P = cre_hbm.shape[1]
    ng, n, Dh, Dm = wo_hbm.shape
    M = mem0_hbm.shape[0]
    L, hs, n_seg = M + seg, seg // 2, S // seg
    na = SSM.n
    ka, kc = D // na, 2 * P // na
    nb, nc = kc // LN, ka // LN
    q1, q2 = n_blk // 4, n_blk // 2
    ppg = (n_blk - q2) // ng
    slabs = wq_hbm.shape[1]
    spp = 6 * slabs // n_blk
    ring = wst_v.shape[2]
    w_parts = ((0, slabs), (slabs, 2 * slabs), (2 * slabs, ring), (ring, 3 * slabs))
    lanes = lambda j: pl.ds(j * LN, LN)
    row = lax.broadcasted_iota(jnp.int32, (8, LN), 0)
    C_F, C_SKIP, C_HOP, C_POW = 0, 2, 3, 9
    SEM_X, SEM_BX, SEM_YA, SEM_YB, SEM_V, SEM_W, SEM_B = 0, 3, 4, 5, 6, 7, 11
    SEM_C = SEM_B + nb
    SEM_WO = SEM_C + nb
    one = pl.program_id(0) + 1

    def region(fn):
        pl.loop(0, one)(fn)

    def by_parity(i, fn):
        for par in range(2):
            pl.when(i % 2 == par)(functools.partial(fn, par))

    staged = lambda lo, hi: wst_v.at[:, :, pl.ds(lo % ring, hi - lo)]

    def w_start(p):
        lo, hi = w_parts[p]
        _start(pltpu.make_async_copy((wq_hbm, wk_hbm, wv_hbm)[lo // slabs].at[:, pl.ds(lo % slabs, hi - lo), r],
                                     staged(lo, hi).at[r % 2, :, :, :, pl.ds(2 * (r // 2), 2)], sems.at[SEM_W + p])
               for r in range(16))

    def w_wait(p):
        pltpu.make_async_copy(staged(*w_parts[p]), staged(*w_parts[p]), sems.at[SEM_W + p]).wait()

    def discretise(lre, lim, log_dt, skip):
        lre, lim = lre.astype(F32), lim.astype(F32)
        dt = jnp.exp(log_dt.astype(F32)).astype(log_dt.dtype).astype(F32)
        mag = jnp.exp(dt * lre)
        a_re, a_im = mag * jnp.cos(dt * lim), mag * jnp.sin(dt * lim)
        big = jnp.maximum(jnp.abs(lre), jnp.abs(lim))
        c, d = lre / big, lim / big
        den = (c * c + d * d) * big
        f_re = 2.0 * ((a_re - 1.0) * c + a_im * d) / den
        f_im = 2.0 * (a_im * c - (a_re - 1.0) * d) / den
        pows = [(a_re, -a_im)]
        for r in range(1, TL):
            pows.append(_cmul(*pows[(r + 1) // 2 - 1], *pows[r // 2]))
        hops = [pows[-1]]
        for _ in range(2):
            hops.append(_cmul(*hops[-1], *hops[-1]))
        for j in range(P // LN):
            bc = lambda v: jnp.broadcast_to(v[j:j + 1], (8, LN))
            coefs = [bc(f_re), bc(-f_im), bc(skip.astype(F32))]
            coefs += [jnp.where(row >= sh, bc(v), 0.0) for sh, hop in zip((1, 2, 4), hops) for v in hop]
            coef_v[j] = jnp.stack(coefs + [bc(v) for p in pows for v in p])

    def product_dots(prod, halves, groups, weight, width):
        halves = functools.cache(halves)
        xi = functools.cache(lambda i: halves(i)[1] - SSM.t[i] * halves(i)[0])
        factor = SSM.left_factors(lambda i: halves(i)[0], xi)
        lhs = functools.cache(lambda slot: factor(slot).astype(BF16))

        def dot(slot, g):
            prod[g, slot] = jnp.dot(lhs(slot), pltpu.bitcast(weight(g, slot).reshape(-1, LN), BF16),
                                    preferred_element_type=F32)

        order = [v for i in range(na) for v in ((SSM.R(i), 1), (SSM.Q(i), 3))]
        order += [v for p in SSM.pairs for v in ((SSM.S(*p), 1.5), (SSM.U(*p), 3), (SSM.L(*p), 3))]
        return [(hb // 8 * (width - 1 + (c * width if g == 0 else 0)), functools.partial(dot, slot, g))
                for slot, c in order for g in range(groups)]

    def x_halves(i, tiles):
        parts = [_halves(pltpu.bitcast(xp_v[i, :, :, lanes(q)].reshape(-1, LN), U32)) for q in tiles]
        return [jnp.concatenate(v, axis=1) for v in zip(*parts)]

    both = lambda i: (i, i // 2)
    states = lambda i, par: (ga_v[par].at[i[1]], gb_v.at[i[0]])

    def scan_units(i, par, plain=None):
        def group(g):
            prod = prod_v[1 if plain else par].at[g]
            blocks = range(g * na // 2, (g + 1) * na // 2)
            coef = functools.cache(lambda j, m: (coef_v[j, m], coef_v[j, m + 1]))
            local, entry = collections.defaultdict(list), {}

            @functools.cache
            def drive(k):
                rows = lambda slot: prod[slot, pl.ds(8 * k, 8), :]
                return [[rows(plain(h, c)) for c in range(na)] for h in range(2)] if plain else SSM.combine(rows)

            def advance(j, k):
                c = 2 * (j - blocks[0])
                fr, fi = coef(j, C_F)
                for h in range(2):
                    vr, vi = drive(k)[h][c:c + 2]
                    vr, vi = vr * fr + vi * fi, vr * fi - vi * fr
                    if local[j]:
                        sr, si = _cmul(*local[j][-1], *coef(j, C_POW))
                        vr, vi = vr + sr, vi + si
                    local[j].append((vr, vi))
                for e, v in enumerate(local[j][-1], c):
                    prod[plain(0, e) if plain else e, pl.ds(8 * k, 8), :] = v

            def finish(j, steps):
                if j not in entry:
                    e = [jnp.where(row == 0, carry_v[j, h], pltpu.roll(local[j][-1][h], 1, 0)) for h in range(2)]
                    for m, sh in enumerate((1, 2, 4)):
                        sr, si = _cmul(pltpu.roll(e[0], sh, 0), pltpu.roll(e[1], sh, 0), *coef(j, C_HOP + 2 * m))
                        e = [e[0] + sr, e[1] + si]
                    entry[j] = e
                for r in steps:
                    at = 8 * (r % 2 * TL // 2 + r // 2)
                    for h, v in enumerate(map(lax.add, local[j][r], _cmul(*entry[j], *coef(j, C_POW + 2 * r)))):
                        states(i, par)[h][at // TL, pl.ds(at % TL, 8), lanes(j)] = v
                        if r == TL - 1:
                            carry_v[j, h] = pltpu.roll(v, 1, 0)

            return ([(28 if plain else 76 - 36 * (j - blocks[0]), functools.partial(advance, j, k))
                     for k in range(TL // 2) for j in blocks]
                    + [(16 + 34 * (r == 0), functools.partial(finish, j, range(r, r + 2)))
                       for r in range(0, TL, 2) for j in blocks])
        return [v for g in range(nb) for v in group(g)]

    def s5_states(vec_v, raw_v, c_v, tr_v, bs_v):
        x_part = (pl.ds(0, 2), pl.ds(2, q1), pl.ds(2 + q1, n_blk - q1 - 2))

        def x_start(p):
            _start(pltpu.make_async_copy(ax_hbm.at[x_part[p], c, pl.ds(2 * k, 2)], xp_v.at[x_part[p], k, pl.ds(2 * c, 2)],
                                         sems.at[SEM_X + p]) for c in range(8) for k in range(TL // 2))

        def x_wait(p):
            pltpu.make_async_copy(xp_v.at[x_part[p]], xp_v.at[x_part[p]], sems.at[SEM_X + p]).wait()

        vec_cp = [pltpu.make_async_copy(w, vec_v.at[i], sems.at[SEM_V])
                  for i, w in enumerate((lre_hbm, lim_hbm, ldt_hbm, dsk_hbm))]
        b_cp = lambda g: [pltpu.make_async_copy(w.at[g], raw_v.at[g, pl.ds(i * n // 2, n // 2)], sems.at[SEM_B + g])
                          for i, w in enumerate((bre_hbm, bim_hbm))]
        c_cp = lambda p: [pltpu.make_async_copy(w.at[:, pl.ds(pl.multiple_of(k + p * LN, LN), LN)], c_v.at[p, i],
                                                sems.at[SEM_C + p])
                          for i, (w, k) in enumerate(itertools.product((cre_hbm, cim_hbm), range(0, P, kc)))]
        wo_cp = lambda p: pltpu.make_async_copy(
            wo_hbm.at[p // ppg, :, pl.ds(pl.multiple_of(p % ppg * (Dh // ppg), Dh // ppg), Dh // ppg)],
            raw_v.at[p], sems.at[SEM_WO + p])

        def turn_units(tile, par):
            def turn(*at):
                tr_v[par][at] = pltpu.bitcast(tile(*at).T, U32)
            return [(24, functools.partial(turn, *at)) for at in itertools.product(range(nc), range(na), range(na))]

        def factor_units(dst, par):
            def load(k, r, i):
                return [(w, _halves(w)) for w in (tr_v[par][k, i, j, pl.ds(r, 8), :] for j in range(na))]

            def store(k, r, slot, v):
                dst[k, slot, pl.ds(r, 8), :] = v
            return [v for at in itertools.product(range(nc), range(0, LN // 2, 8))
                    for v in SSM.right_factor_units(functools.partial(load, *at), functools.partial(store, *at))]

        def wo_units(p):
            def load(r, i):
                return [(w, _halves(w)) for w in (pltpu.bitcast(raw_v[p, i, pl.ds(r, 16), lanes(j)], U32) for j in range(n))]

            def store(r, slot, v):
                wo_v[p, slot, pl.ds(r // 2, 8), :] = v
            return [v for r in range(0, Dh // ppg, 16)
                    for v in ATT.right_factor_units(functools.partial(load, r), functools.partial(store, r))]

        b_block = lambda g, j, cols: raw_v[g, pl.ds(j % 2 * n // 2 + j // 2 * ppg, ppg), :, cols].reshape(LN, -1)
        b_turns = lambda g, par: turn_units(lambda k, i, j: b_block(g, j, lanes(i * nc + k)), par)
        c_turns = lambda p, par: turn_units(lambda k, i, j: c_v[p, i, lanes(k * na + j), :], par)
        state_dots = lambda i, par: product_dots(prod_v[par], lambda k: x_halves(i, range(k * nc, (k + 1) * nc)), nb,
                                                 lambda g, slot: bs_v[g, :, slot], nc)

        def sweep(i, *extra):
            prev = both(i - 1)
            by_parity(i, lambda par: _weave(state_dots(i, par), scan_units(prev, 1 - par), *(e(par) for e in extra)))

        _start(vec_cp)
        x_start(0)
        for g in range(nb):
            _start(b_cp(g))
        for buf in (carry_v, tr_v[1], o_v[1], *po_v):
            buf[...] = jnp.zeros_like(buf)
        _wait(vec_cp)
        discretise(*(vec_v[i] for i in range(4)))
        x_wait(0)

        lhs = [[v.astype(BF16) for v in x_halves(i, range(D // LN))] for i in range(2)]
        plain = lambda i, h, j: (2 * i + h) * na + j

        def first_blocks(g, par, *extra):
            raw = functools.cache(lambda j: b_block(g, j, slice(None)))

            def dot(i, h, j):
                prod_v[1][g, plain(i, h, j)] = lax.dot_general(lhs[i][h], raw(j), NT, preferred_element_type=F32)
            _weave([(56 + 64 * (i + h == 0), functools.partial(dot, i, h, j))
                    for j in range(na) for i in range(2) for h in range(2)],
                   b_turns(g, par), *extra)

        @pl.loop(0, nb)
        def _(g):
            _wait(b_cp(g))

            @pl.when(g == nb - 1)
            def _():
                x_start(1)
                for p in range(nb):
                    _start(c_cp(p))
            prev = jnp.maximum(g - 1, 0)
            by_parity(g, lambda par: first_blocks(g, par, factor_units(bs_v.at[prev], 1 - par)))

        for _, unit in factor_units(bs_v.at[nb - 1], (nb - 1) % 2):
            unit()
        x_wait(1)
        region(lambda _: _weave(state_dots(2, 0),
                                [v for i in range(2) for v in scan_units(both(i), i, functools.partial(plain, i))]))

        @pl.loop(q1 - 1, q2)
        def _(i):
            @pl.when(i == q1)
            def _():
                x_start(2)
                _start(wo_cp(p) for p in range(ng * ppg))
            pl.when(i == 2 + q1)(lambda: x_wait(2))
            pl.when(i + 1 < q2)(lambda: _wait(c_cp(i + 1 - q1)))
            now, ahead = jnp.maximum(i - q1, 0), jnp.minimum(i + 1, q2 - 1) - q1
            sweep(i, functools.partial(factor_units, cs_v.at[now]), lambda par: c_turns(ahead, 1 - par))

        @pl.loop(q2, n_blk)
        def _(i):
            p = i - q2
            pl.when(i == n_blk - 5)(lambda: w_start(0))
            pl.when(i == n_blk - 1)(lambda: w_start(1))
            wo_cp(p).wait()
            sweep(i, lambda par: wo_units(p))

    def output_dots(i, par):
        def halves(k):
            src, cols = states(i, par)[k * kc // P], pl.ds(k * kc % P, kc)
            return [src[pl.ds(4 * h, 4), :, cols].reshape(hb, kc) for h in range(2)]
        return product_dots(prod_v[par], halves, nc, lambda g, slot: cs_v[:, g, slot], nb)

    def output_units(i, par):
        total = functools.cache(lambda g, k: SSM.combine(lambda slot: prod_v[par][g, slot, pl.ds(8 * k, 8), :]))

        def unit(k, q):
            x = _halves(pltpu.bitcast(xp_v[i[0], k, :, lanes(q)], U32))
            ga_v[par][i[1], k, :, lanes(q)] = jnp.concatenate(
                [y[q % na] + v * coef_v[q, C_SKIP] for y, v in zip(total(q // na, k), x)], axis=0)
        return [(28 - 6 * j, functools.partial(unit, k, g * na + j))
                for g in range(nc) for k in range(TL // 2) for j in range(na)]

    def qkv_units(first, first_staged, par):
        src, dst = wst_v.at[:, :, pl.ds(first_staged, spp)], wqkv_v.at[pl.ds(first, spp)]

        def load(u, g, i):
            out = []
            for jp in range(g * n // 2, (g + 1) * n // 2):
                even, odd = (pltpu.bitcast(src[h, i, u, jp], U32) for h in range(2))
                words = (even & jnp.uint32(0xFFFF)) | (odd << 16), (even >> 16) | (odd & jnp.uint32(0xFFFF0000))
                out += zip(words, zip(_halves(even), _halves(odd)))
            return out

        def store(u, g, slot, v):
            dst[u, g, slot] = v
        return [v for at in list(itertools.product(range(spp), range(ng)))[par::2]
                for v in ATT.right_factor_units(functools.partial(load, *at), functools.partial(store, *at))]

    def s5_outputs_and_attention(bx_v, mem0_v, mem_v, pq_v):
        x_cp = [pltpu.make_async_copy(a, b, sems.at[SEM_BX]) for a, b in ((bx_hbm, bx_v), (mem0_hbm, mem0_v))]
        ya_cp = [pltpu.make_async_copy(ga_v[par].at[:, r // 2, pl.ds(r % 2 * 8, 8)],
                                       out_hbm.at[:, par, :, r, pl.ds(0, D)], sems.at[SEM_YA])
                 for par in range(2) for r in range(TL)]
        pair_rows = lambda k: (2 * seg * k // tb, pl.ds(2 * seg * k % tb // TL, 2 * seg // TL))

        def yb_start(k):
            blk, rows = pair_rows(k)
            pltpu.make_async_copy(gb_v.at[blk, rows], out_hbm.at[blk // 2, blk % 2, rows, :, pl.ds(D, Dm)],
                                  sems.at[SEM_YB]).start()

        w_wait(0)
        region(lambda i: _weave(output_dots(both(0), 0), scan_units(both(n_blk - 1), 1), qkv_units(i, 0, 0)))

        @pl.loop(1, n_blk)
        def _(i):
            for p in range(1, len(w_parts)):
                @pl.when(i == w_parts[p][0] // spp * 2)
                def _():
                    if p == 1:
                        w_start(2)
                        w_start(3)
                        _start(x_cp)
                    w_wait(p)
            cur, prev, at = both(i), both(jnp.maximum(i - 1, 0)), (i // 2 * spp, i // 2 * spp % ring)
            by_parity(i, lambda par: _weave(output_dots(cur, par), output_units(prev, 1 - par), qkv_units(*at, par)))

        _wait(x_cp)
        scale = float(Dh) ** -0.5
        key = lax.broadcasted_iota(jnp.int32, (L, L), 0)
        query = lax.broadcasted_iota(jnp.int32, (L, L), 1)
        mask = (query < M) | (query >= key)
        symmetric = [ATT.S(*p) for p in ATT.pairs]
        by_last = sorted(ATT.pairs, key=lambda p: p[::-1])
        qkv_order = list(range(n // 2)) + by_last[:2 * n] + list(range(n // 2, n)) + by_last[2 * n:]
        wo_order = list(range(n)) + ATT.pairs
        carried = [[s for s in ATT.half_slots(odd, wo_order, 1) if s not in symmetric] for odd in range(2)]
        qkv_weight = lambda w, g, slot: pltpu.bitcast(wqkv_v[pl.ds(w * slabs, slabs), g, slot].reshape(-1, LN), BF16)
        wo_weight = lambda slot, g0, g1: pltpu.bitcast(wo_v[pl.ds(g0 * ppg, (g1 - g0) * ppg), slot].reshape(-1, LN), BF16)

        def step_lhs(odd, slot, mem, own, other):
            rows = [ATT.single_factor(odd, mem, slot), own(slot)] + ([] if slot in symmetric else [other(slot)])
            return jnp.concatenate(rows, axis=0)

        def token_factors(s):
            rows = bx_v.at[pl.ds(pl.multiple_of(s * seg, seg), seg)]
            x1, x2 = (functools.cache(lambda i, r=r: rows[pl.ds(r, hs), lanes(i)].astype(F32)) for r in (0, hs))
            return ATT.left_factors(x1, functools.cache(lambda i: x2(i) - ATT.t[i] * x1(i)))

        def head_factors(odd, g0, g1):
            mem, x1, xi = (functools.cache(lambda i, r=r: o_v[odd][i, r, pl.ds(g0 * Dh, (g1 - g0) * Dh)])
                           for r in (pl.ds(0, M), pl.ds(M, hs), pl.ds(M + hs, hs)))
            return mem, ATT.left_factors(x1, xi)

        def store_segment(at, odd):
            for r in range(0, hs, 8):
                for j, y in enumerate(zip(*ATT.combine(lambda slot: po_v[odd][slot, pl.ds(r, 8), :]))):
                    gb_v.at[at][pl.ds(2 * odd, 2), pl.ds(r, 8), lanes(j)] = jnp.stack(y)

        def pair_of_steps(k):
            events = collections.defaultdict(list)
            clock = [0]

            def dot(lhs, rhs):
                while events and min(events) <= clock[0]:
                    for fn in events.pop(min(events)):
                        fn()
                clock[0] += rhs.shape[0] // LN
                return jnp.dot(lhs(), rhs, preferred_element_type=F32)

            def later(fn, g, delays):
                for delay, j in zip(delays, range(0, n, N_MXU), strict=True):
                    events[clock[0] + delay].append(functools.partial(fn, g, range(j, j + N_MXU)))

            def step(odd, own, ahead):
                store_segment(done, odd)
                mem = functools.cache(lambda i: mem_v[:, lanes(i)])
                lhs = functools.cache(lambda slot: step_lhs(odd, slot, mem, own, ahead))
                qkv, prob = {}, {}

                def project(g, w):
                    m = {}
                    for slot in ATT.half_slots(odd, qkv_order, N_MXU):
                        m[slot] = dot(lambda: lhs(slot), qkv_weight(w, g, slot))
                        if slot not in symmetric:
                            pq_v[odd][w, g, carried[odd].index(slot)] = m[slot][M + hs:]
                    parts = (ATT.single_combine(odd, lambda slot: m[slot][:M], qkv_order),
                             *ATT.combine(lambda slot: m[slot][M:M + hs] if slot in m
                                          else pq_v[1 - odd][w, g, carried[1 - odd].index(slot)], qkv_order))
                    for j, rows in enumerate(zip(*parts)):
                        qkv[g, j, w] = jnp.concatenate(rows, axis=0).astype(BF16 if w == 2 else F32)

                def softmax(g, heads):
                    for j in heads:
                        z = lax.dot_general(qkv.pop((g, j, 1)), qkv.pop((g, j, 0)), NT, preferred_element_type=F32)
                        z = jnp.where(mask, z * (scale * LOG2_E), -1e9 * LOG2_E)
                        e = jnp.exp2(z - jnp.max(z, axis=0, keepdims=True))
                        prob[g, j] = (e * pl.reciprocal(jnp.sum(e, axis=0, keepdims=True), full_range=False)).T

                def mix(g, heads):
                    for j in heads:
                        o = jnp.dot(prob.pop((g, j)), qkv.pop((g, j, 2)), preferred_element_type=F32)
                        o_v[odd][j, :, lanes(g)] = jnp.concatenate(
                            [o[:M + hs], o[M + hs:] - ATT.t[j] * o[M:M + hs]], axis=0)

                for g in range(ng):
                    project(g, 0)
                    project(g, 1)
                    later(softmax, g, (12, 36))
                    project(g, 2)
                    later(mix, g, (12, 16) if g < ng - 1 else (48, 72))

                heads = functools.cache(head_factors)
                part = lambda slot, g0, g1: dot(
                    lambda: step_lhs(odd, slot, *heads(odd, g0, g1), heads(1 - odd, g0, g1)[1]), wo_weight(slot, g0, g1))
                m = {slot: part(slot, 0, ng // 2) for slot in ATT.half_slots(odd, wo_order, 2)}
                for slot in m:
                    m[slot] = part(slot, ng // 2, ng) + m[slot]
                    po_v[odd][slot] = m[slot][M:M + hs]
                    if slot not in symmetric:
                        po_v[1 - odd][slot] = m[slot][M + hs:]
                for j, v in enumerate(ATT.single_combine(odd, lambda slot: m[slot][:M], wo_order)):
                    mem_v[:, lanes(j)] = v

            done = pair_rows(jnp.maximum(k - 1, 0))
            tokens = [token_factors(s) for s in (2 * k, 2 * k + 1, jnp.minimum(2 * k + 2, n_seg - 1))]
            step(0, *tokens[:2])
            step(1, *tokens[1:])
            assert not events
            pl.when(k > 0)(lambda: yb_start(k - 1))

        def before_first_step(_):
            first = token_factors(0)
            mem_v[...] = mem0_v[...].astype(F32)

            def dot(w, g, a):
                pq_v[1][w, g, a] = jnp.dot(first(carried[1][a]), qkv_weight(w, g, carried[1][a]),
                                           preferred_element_type=F32)
            _weave([(2, functools.partial(dot, *at))
                    for at in itertools.product(range(3), range(ng), range(len(carried[1])))],
                   output_units(both(n_blk - 1), 1))

        def after_last_step(_):
            last = head_factors(1, 0, ng)[1]
            for a, slot in enumerate(carried[0]):
                po_v[1][slot] = jnp.dot(last(slot), wo_weight(slot, 0, ng), preferred_element_type=F32)
                if a == n:
                    store_segment(pair_rows(n_seg // 2 - 1), 0)
            store_segment(pair_rows(n_seg // 2 - 1), 1)

        region(before_first_step)
        _start(ya_cp)
        pl.loop(0, n_seg // 2)(pair_of_steps)
        region(after_last_step)
        yb_start(n_seg // 2 - 1)
        _wait(ya_cp)
        pltpu.make_async_copy(gb_v, gb_v, sems.at[SEM_YB]).wait()

    pl.run_scoped(
        s5_states, pltpu.VMEM((4, P // LN, LN), BF16), pltpu.VMEM((ng * ppg, n, Dh // ppg, Dm), BF16),
        pltpu.VMEM((nb, na, D, LN), BF16), [pltpu.VMEM((nc, na, na, LN // 2, LN), U32)] * 2,
        pltpu.VMEM((nb, nc, SSM.slots, LN // 2, LN), U32))
    pl.run_scoped(
        s5_outputs_and_attention, pltpu.VMEM((S, Dm), BF16), pltpu.VMEM((M, Dm), BF16), pltpu.VMEM((M, Dm), F32),
        [pltpu.VMEM((3, ng, n + len(ATT.pairs), hs, Dh), F32)] * 2)


@functools.partial(jax.jit, static_argnames=("B_seg_len",))
def pallas_concat_heads__ssm_conv_s5__memory_aug_recurrent_mem_tr__prompt_kernel(
    A_x, A_Lambda_re, A_Lambda_im, A_B_re, A_B_im, A_C_re, A_C_im, A_log_dt, A_Dskip,
    B_x, B_mem0, B_Wq, B_Wk, B_Wv, B_Wo, B_seg_len,
):
    batch, S, D = A_x.shape
    P = A_B_re.shape[0]
    Dm, H, Dh = B_Wq.shape
    M = B_mem0.shape[1]
    seg = B_seg_len
    assert (batch, S, D, P, Dm, H, Dh, M, seg) == (1, 2048, 1024, 1024, 1024, 32, 128, 8, 32)
    n, ng, n_blk = ATT.n, H // ATT.n, S // (8 * TL)
    nb, nc = 2 * P // (SSM.n * LN), D // (SSM.n * LN)
    slabs = Dm // (n * 16)
    hbm = pl.BlockSpec(memory_space=pl.ANY)
    vec = lambda v: v.reshape(-1, LN)
    out = pl.pallas_call(
        functools.partial(_kernel, seg=seg),
        out_shape=jax.ShapeDtypeStruct((n_blk // 2, 2, 8, TL, D + Dm), F32),
        grid=(1,),
        in_specs=[hbm] * 15,
        out_specs=hbm,
        scratch_shapes=[
            pltpu.VMEM((n_blk, TL // 2, 16, D), BF16),
            pltpu.VMEM((nb, nc, SSM.slots, LN // 2, LN), U32),
            pltpu.VMEM((2, n, 2 * slabs + 2, H // 2, 16, Dh), BF16),
            pltpu.VMEM((3 * slabs, ng, ATT.slots, 8, Dh), U32),
            pltpu.VMEM((n_blk // 2, ATT.slots, ng * Dh // n_blk, LN), U32),
            [pltpu.VMEM((n_blk // 2, 8, TL, P), F32)] * 2,
            pltpu.VMEM((n_blk, 8, TL, P), F32),
            [pltpu.VMEM((nb, SSM.slots, 4 * TL, LN), F32)] * 2,
            pltpu.VMEM((P // LN, 9 + 2 * TL, 8, LN), F32),
            pltpu.VMEM((P // LN, 2, 8, LN), F32),
            [pltpu.VMEM((n, M + seg, ng * Dh), F32)] * 2,
            [pltpu.VMEM((ATT.slots, seg // 2, LN), F32)] * 2,
            pltpu.SemaphoreType.DMA((11 + 2 * nb + n_blk // 2,)),
        ],
        compiler_params=pltpu.CompilerParams(vmem_limit_bytes=127 * 2**20),
        name="fused_s5_rmt",
    )(A_x.reshape(n_blk, 8, TL, D), vec(A_Lambda_re), vec(A_Lambda_im),
      A_B_re.reshape(nb, n // 2, -1, D), A_B_im.reshape(nb, n // 2, -1, D), A_C_re, A_C_im,
      vec(A_log_dt), vec(A_Dskip), B_x.reshape(S, Dm), B_mem0.reshape(M, Dm),
      *(w.reshape(n, slabs, 16, H // 2, 2, Dh) for w in (B_Wq, B_Wk, B_Wv)),
      B_Wo.reshape(ng, n, Dh, Dm))
    return out.reshape(1, S, D + Dm)
```

```python
import collections
import functools
import itertools

import jax
import jax.numpy as jnp
from jax import lax
import jax.experimental.pallas as pl
import jax.experimental.pallas.tpu as pltpu

F32 = jnp.float32
BF16 = jnp.bfloat16
U32 = jnp.uint32
NT = (((1,), (1,)), ((), ()))
LN = 128
TL = 16
N_MXU = 4
LOG2_E = 1.4426950408889634


class _Scheme:
    def __init__(self, slopes):
        self.t = slopes
        self.n = n = len(slopes)
        self.pairs = list(itertools.combinations(range(n), 2))
        self.slots = 2 * n + 3 * len(self.pairs)

    def R(self, i): return i
    def Q(self, i): return self.n + i
    def S(self, i, j): return 2 * self.n + self.pairs.index((i, j))
    def U(self, i, j): return self.S(i, j) + len(self.pairs)
    def L(self, i, j): return self.U(i, j) + len(self.pairs)

    def pair(self, slot):
        return self.pairs[(slot - 2 * self.n) % len(self.pairs)]

    def left_factors(self, x1, xi):
        @functools.cache
        def factor(slot):
            if slot < 2 * self.n:
                return x1(slot) if slot < self.n else xi(slot - self.n)
            i, j = self.pair(slot)
            d = self.t[i] - self.t[j]
            if slot == self.S(i, j):
                return xi(i) + xi(j)
            if slot == self.U(i, j):
                return factor(self.S(i, j)) + d * x1(i)
            return factor(self.S(i, j)) - d * x1(j)
        return factor

    def combine(self, m, order=None):
        y1, rest = [None] * self.n, [None] * self.n
        for item in order or list(range(self.n)) + self.pairs:
            if isinstance(item, tuple):
                i, j = item
                u, l = m(self.U(i, j)), m(self.L(i, j))
                e = (m(self.S(i, j)) - u - l) * (1.0 / (self.t[i] - self.t[j]))
                _add(y1, i, e)
                _add(y1, j, e, -1)
                _add(rest, j, u)
                _add(rest, i, l)
            else:
                _add(y1, item, m(self.R(item)))
                _add(rest, item, m(self.Q(item)))
        return y1, [rest[j] + self.t[j] * y1[j] for j in range(self.n)]

    def half_slots(self, odd, order, batch):
        slots, pend = [], []
        for item in order:
            if isinstance(item, tuple):
                pend.append(item)
                if len(pend) == batch:
                    slots += [self.S(*p) for p in pend] + [(self.L if odd else self.U)(*p) for p in pend]
                    pend = []
            else:
                slots.append((self.Q if odd else self.R)(item))
        assert not pend
        return slots

    def single_factor(self, odd, a, slot):
        if slot < 2 * self.n:
            return a(slot % self.n)
        i, j = self.pair(slot)
        return a(j) if slot == self.S(i, j) and not odd else a(i) + a(j)

    def single_combine(self, odd, m, order):
        y = [None] * self.n
        for item in order:
            if isinstance(item, tuple):
                i, j = item
                side = m((self.L if odd else self.U)(i, j))
                d = m(self.S(i, j)) - side
                _add(y, i, side if odd else d)
                _add(y, j, d, 1 if odd else -1)
            else:
                _add(y, item, m((self.Q if odd else self.R)(item)))
        return y

    def right_factor_units(self, load, store):
        rows = {}

        def block_row(i):
            rows[i] = load(i)
            for j, (word, _) in enumerate(rows[i]):
                if j != i:
                    store(self.U(i, j) if i < j else self.L(j, i), word)
            store(self.R(i), _round_pack(*(functools.reduce(lax.add, [v[1][h] for v in rows[i]]) for h in range(2))))

        def symmetric(i, j):
            store(self.S(i, j), _round_pack(*map(lax.add, _halves(rows[i][j][0]), rows[j][i][1])))

        def block_column(j):
            wide = lambda i: pltpu.bitcast(rows[i][j][0], BF16).astype(F32)
            total = functools.reduce(lax.sub, [wide(j)] + [wide(i) for i in range(self.n) if i != j])
            store(self.Q(j), pltpu.bitcast(total.astype(BF16), U32))

        units = []
        for j in range(self.n):
            units += [(6 * self.n + 4, functools.partial(block_row, j))]
            units += [(10, functools.partial(symmetric, i, j)) for i in range(j)]
        return units + [(4 * self.n + 3, functools.partial(block_column, j)) for j in range(self.n)]


SSM = _Scheme((-1.375, -0.375, 0.375, 1.375))
ATT = _Scheme((-2.25, -1.125, -0.5625, -0.1875, 0.1875, 0.5625, 1.125, 2.25))


def _add(acc, i, v, sign=1):
    if acc[i] is None:
        acc[i] = v if sign > 0 else -v
    else:
        acc[i] = acc[i] + v if sign > 0 else acc[i] - v


def _cmul(ar, ai, br, bi):
    return ar * br - ai * bi, ar * bi + ai * br


def _halves(word):
    return pltpu.bitcast(word << 16, F32), pltpu.bitcast(word & jnp.uint32(0xFFFF0000), F32)


def _round_pack(lo, hi):
    bits = pltpu.bitcast(jnp.concatenate([lo, hi], axis=1).astype(BF16).astype(F32), U32)
    return (bits[:, :LN] >> 16) | bits[:, LN:]


def _weave(dots, *streams):
    side = []
    for units in streams:
        total, seen = sum(c for c, _ in units), 0
        for c, fn in units:
            side.append(((seen + c / 2) / total, c, fn))
            seen += c
    side.sort(key=lambda v: v[0])
    rate = (sum(c for c, _ in dots) + sum(v[1] for v in side)) / len(dots)
    spent = 0
    for k, (c, fn) in enumerate(dots):
        fn()
        spent += c
        while side and (spent + side[0][1] / 2 <= rate * (k + 1) or k + 1 == len(dots)):
            _, c, fn = side.pop(0)
            fn()
            spent += c


def _start(copies):
    for cp in copies:
        cp.start()


def _wait(copies):
    for cp in copies:
        cp.wait()


def _kernel(
    ax_hbm, lre_hbm, lim_hbm, bre_hbm, bim_hbm, cre_hbm, cim_hbm, ldt_hbm, dsk_hbm,
    bx_hbm, mem0_hbm, wq_hbm, wk_hbm, wv_hbm, wo_hbm,
    out_hbm,
    xp_v, cs_v, wst_v, wqkv_v, wo_v, ga_v, gb_v, prod_v, coef_v, carry_v, o_v, po_v, sems,
    *, seg,
):
    n_blk, _, _, D = ax_hbm.shape
    tb, hb = 8 * TL, 4 * TL
    S = n_blk * tb
    P = cre_hbm.shape[-1]
    ng, n, Dh, Dm = wo_hbm.shape
    M = mem0_hbm.shape[0]
    L, hs, n_seg = M + seg, seg // 2, S // seg
    na = SSM.n
    ka, kc = D // na, 2 * P // na
    nb, nc = kc // LN, ka // LN
    q1, q2 = n_blk // 4, n_blk // 2
    ppg = (n_blk - q2) // ng
    slabs = wq_hbm.shape[1]
    spp = 6 * slabs // n_blk
    ring = wst_v.shape[2]
    w_parts = ((0, slabs), (slabs, 2 * slabs), (2 * slabs, ring), (ring, 3 * slabs))
    lanes = lambda j: pl.ds(j * LN, LN)
    row = lax.broadcasted_iota(jnp.int32, (8, LN), 0)
    C_F, C_SKIP, C_HOP, C_POW = 0, 2, 3, 9
    SEM_X, SEM_BX, SEM_YA, SEM_YB, SEM_V, SEM_W, SEM_B = 0, 3, 4, 5, 6, 7, 11
    SEM_C = SEM_B + nb
    SEM_WO = SEM_C + nb
    one = pl.program_id(0) + 1

    def region(fn):
        pl.loop(0, one)(fn)

    def by_parity(i, fn):
        for par in range(2):
            pl.when(i % 2 == par)(functools.partial(fn, par))

    staged = lambda lo, hi: wst_v.at[:, :, pl.ds(lo % ring, hi - lo)]

    def w_start(p):
        lo, hi = w_parts[p]
        _start(pltpu.make_async_copy((wq_hbm, wk_hbm, wv_hbm)[lo // slabs].at[:, pl.ds(lo % slabs, hi - lo), r],
                                     staged(lo, hi).at[r % 2, :, :, :, pl.ds(2 * (r // 2), 2)], sems.at[SEM_W + p])
               for r in range(16))

    def w_wait(p):
        pltpu.make_async_copy(staged(*w_parts[p]), staged(*w_parts[p]), sems.at[SEM_W + p]).wait()

    def discretise(lre, lim, log_dt, skip):
        lre, lim = lre.astype(F32), lim.astype(F32)
        dt = jnp.exp(log_dt.astype(F32)).astype(log_dt.dtype).astype(F32)
        mag = jnp.exp(dt * lre)
        a_re, a_im = mag * jnp.cos(dt * lim), mag * jnp.sin(dt * lim)
        big = jnp.maximum(jnp.abs(lre), jnp.abs(lim))
        c, d = lre / big, lim / big
        den = (c * c + d * d) * big
        f_re = 2.0 * ((a_re - 1.0) * c + a_im * d) / den
        f_im = 2.0 * (a_im * c - (a_re - 1.0) * d) / den
        pows = [(a_re, -a_im)]
        for r in range(1, TL):
            pows.append(_cmul(*pows[(r + 1) // 2 - 1], *pows[r // 2]))
        hops = [pows[-1]]
        for _ in range(2):
            hops.append(_cmul(*hops[-1], *hops[-1]))
        for j in range(P // LN):
            bc = lambda v: jnp.broadcast_to(v[j:j + 1], (8, LN))
            coefs = [bc(f_re), bc(-f_im), bc(skip.astype(F32))]
            coefs += [jnp.where(row >= sh, bc(v), 0.0) for sh, hop in zip((1, 2, 4), hops) for v in hop]
            for m, v in enumerate(coefs + [bc(v) for p in pows for v in p]):
                coef_v[j, m] = v

    def product_dots(prod, halves, groups, weight, width):
        halves = functools.cache(halves)
        xi = functools.cache(lambda i: halves(i)[1] - SSM.t[i] * halves(i)[0])
        factor = SSM.left_factors(lambda i: halves(i)[0], xi)
        lhs = functools.cache(lambda slot: factor(slot).astype(BF16))

        def dot(slot, g):
            prod[g, slot] = jnp.dot(lhs(slot), pltpu.bitcast(weight(g, slot).reshape(-1, LN), BF16),
                                    preferred_element_type=F32)

        order = [v for i in range(na) for v in ((SSM.R(i), 1), (SSM.Q(i), 3))]
        order += [v for p in SSM.pairs for v in ((SSM.S(*p), 1.5), (SSM.U(*p), 3), (SSM.L(*p), 3))]
        return [(hb // 8 * (width - 1 + (c * width if g == 0 else 0)), functools.partial(dot, slot, g))
                for slot, c in order for g in range(groups)]

    def x_halves(i, tiles):
        parts = [_halves(pltpu.bitcast(xp_v[i, :, :, lanes(q)].reshape(-1, LN), U32)) for q in tiles]
        return [jnp.concatenate(v, axis=1) for v in zip(*parts)]

    both = lambda i: (i, i // 2)
    states = lambda i, par: (ga_v[par].at[i[1]], gb_v.at[i[0]])

    def scan_units(i, par, plain=None):
        def group(g):
            prod = prod_v[1 if plain else par].at[g]
            blocks = range(g * na // 2, (g + 1) * na // 2)
            coef = functools.cache(lambda j, m: (coef_v[j, m], coef_v[j, m + 1]))
            local, entry = collections.defaultdict(list), {}

            @functools.cache
            def drive(k):
                rows = lambda slot: prod[slot, pl.ds(8 * k, 8), :]
                return [[rows(plain(h, c)) for c in range(na)] for h in range(2)] if plain else SSM.combine(rows)

            def advance(j, k):
                c = 2 * (j - blocks[0])
                fr, fi = coef(j, C_F)
                for h in range(2):
                    vr, vi = drive(k)[h][c:c + 2]
                    vr, vi = vr * fr + vi * fi, vr * fi - vi * fr
                    if local[j]:
                        sr, si = _cmul(*local[j][-1], *coef(j, C_POW))
                        vr, vi = vr + sr, vi + si
                    local[j].append((vr, vi))
                for e, v in enumerate(local[j][-1], c):
                    prod[plain(0, e) if plain else e, pl.ds(8 * k, 8), :] = v

            def finish(j, steps):
                if j not in entry:
                    e = [jnp.where(row == 0, carry_v[j, h], pltpu.roll(local[j][-1][h], 1, 0)) for h in range(2)]
                    for m, sh in enumerate((1, 2, 4)):
                        sr, si = _cmul(pltpu.roll(e[0], sh, 0), pltpu.roll(e[1], sh, 0), *coef(j, C_HOP + 2 * m))
                        e = [e[0] + sr, e[1] + si]
                    entry[j] = e
                for r in steps:
                    at = 8 * (r % 2 * TL // 2 + r // 2)
                    for h, v in enumerate(map(lax.add, local[j][r], _cmul(*entry[j], *coef(j, C_POW + 2 * r)))):
                        states(i, par)[h][at // TL, pl.ds(at % TL, 8), lanes(j)] = v
                        if r == TL - 1:
                            carry_v[j, h] = pltpu.roll(v, 1, 0)

            return ([(28 if plain else 76 - 36 * (j - blocks[0]), functools.partial(advance, j, k))
                     for k in range(TL // 2) for j in blocks]
                    + [(16 + 34 * (r == 0), functools.partial(finish, j, range(r, r + 2)))
                       for r in range(0, TL, 2) for j in blocks])
        return [v for g in range(nb) for v in group(g)]

    def s5_states(vec_v, raw_v, tr_v, bs_v):
        x_part = (pl.ds(0, 2), pl.ds(2, q1), pl.ds(2 + q1, n_blk - q1 - 2))

        def x_start(p):
            _start(pltpu.make_async_copy(ax_hbm.at[x_part[p], c, pl.ds(2 * k, 2)], xp_v.at[x_part[p], k, pl.ds(2 * c, 2)],
                                         sems.at[SEM_X + p]) for c in range(8) for k in range(TL // 2))

        def x_wait(p):
            pltpu.make_async_copy(xp_v.at[x_part[p]], xp_v.at[x_part[p]], sems.at[SEM_X + p]).wait()

        vec_cp = [pltpu.make_async_copy(w, vec_v.at[i], sems.at[SEM_V])
                  for i, w in enumerate((lre_hbm, lim_hbm, ldt_hbm, dsk_hbm))]
        b_cp = lambda g: [pltpu.make_async_copy(w.at[g], raw_v.at[g, pl.ds(i * n // 2, n // 2)], sems.at[SEM_B + g])
                          for i, w in enumerate((bre_hbm, bim_hbm))]
        c_cp = lambda p: [pltpu.make_async_copy(w.at[k, :, :, pl.ds(pl.multiple_of(c + p * LN, LN), LN)],
                                                raw_v.at[nb + p, :, :, lanes(i * nc + k)], sems.at[SEM_C + p])
                          for i, (w, c) in enumerate(itertools.product((cre_hbm, cim_hbm), range(0, P, kc)))
                          for k in range(nc)]
        wo_cp = lambda p: pltpu.make_async_copy(
            wo_hbm.at[p // ppg, :, pl.ds(pl.multiple_of(p % ppg * (Dh // ppg), Dh // ppg), Dh // ppg)],
            raw_v.at[p], sems.at[SEM_WO + p])

        def turn_units(tile, par):
            def turn(*at):
                tr_v[par][at] = pltpu.bitcast(tile(*at).T, U32)
            return [(24, functools.partial(turn, *at)) for at in itertools.product(range(nc), range(na), range(na))]

        def factor_units(dst, par):
            def load(k, r, i):
                return [(w, _halves(w)) for w in (tr_v[par][k, i, j, pl.ds(r, 8), :] for j in range(na))]

            def store(k, r, slot, v):
                dst[k, slot, pl.ds(r, 8), :] = v
            return [v for at in itertools.product(range(nc), range(0, LN // 2, 8))
                    for v in SSM.right_factor_units(functools.partial(load, *at), functools.partial(store, *at))]

        def wo_units(p):
            def load(r, i):
                return [(w, _halves(w)) for w in (pltpu.bitcast(raw_v[p, i, pl.ds(r, 16), lanes(j)], U32) for j in range(n))]

            def store(r, slot, v):
                wo_v[p, slot, pl.ds(r // 2, 8), :] = v
            return [v for r in range(0, Dh // ppg, 16)
                    for v in ATT.right_factor_units(functools.partial(load, r), functools.partial(store, r))]

        b_block = lambda g, j, cols: raw_v[g, pl.ds(j % 2 * n // 2 + j // 2 * ppg, ppg), :, cols].reshape(LN, -1)
        b_turns = lambda g, par: turn_units(lambda k, i, j: b_block(g, j, lanes(i * nc + k)), par)
        c_turns = lambda p, par: turn_units(
            lambda k, i, j: raw_v[nb + p, pl.ds(j * ppg, ppg), :, lanes(i * nc + k)].reshape(LN, LN), par)
        state_dots = lambda i, par: product_dots(prod_v[par], lambda k: x_halves(i, range(k * nc, (k + 1) * nc)), nb,
                                                 lambda g, slot: bs_v[g, :, slot], nc)

        def sweep(i, *extra):
            prev = both(i - 1)
            by_parity(i, lambda par: _weave(state_dots(i, par), scan_units(prev, 1 - par), *(e(par) for e in extra)))

        _start(vec_cp)
        x_start(0)
        for g in range(nb):
            _start(b_cp(g))
        for buf in (carry_v, tr_v[1], o_v[1], *po_v):
            buf[...] = jnp.zeros_like(buf)
        _wait(vec_cp)
        discretise(*(vec_v[i] for i in range(4)))
        x_wait(0)

        lhs = [[v.astype(BF16) for v in x_halves(i, range(D // LN))] for i in range(2)]
        plain = lambda i, h, j: (2 * i + h) * na + j

        def first_blocks(g, par, *extra):
            raw = functools.cache(lambda j: b_block(g, j, slice(None)))

            def dot(i, h, j):
                prod_v[1][g, plain(i, h, j)] = lax.dot_general(lhs[i][h], raw(j), NT, preferred_element_type=F32)
            _weave([(56 + 64 * (i + h == 0), functools.partial(dot, i, h, j))
                    for j in range(na) for i in range(2) for h in range(2)],
                   b_turns(g, par), *extra)

        @pl.loop(0, nb)
        def _(g):
            _wait(b_cp(g))

            @pl.when(g == nb - 1)
            def _():
                x_start(1)
                for p in range(nb):
                    _start(c_cp(p))
            prev = jnp.maximum(g - 1, 0)
            by_parity(g, lambda par: first_blocks(g, par, factor_units(bs_v.at[prev], 1 - par)))

        for _, unit in factor_units(bs_v.at[nb - 1], (nb - 1) % 2):
            unit()
        x_wait(1)
        region(lambda _: _weave(state_dots(2, 0),
                                [v for i in range(2) for v in scan_units(both(i), i, functools.partial(plain, i))]))

        @pl.loop(q1 - 1, q2)
        def _(i):
            @pl.when(i == q1)
            def _():
                x_start(2)
                _start(wo_cp(p) for p in range(nb))
            pl.when(i == 2 + q1)(lambda: x_wait(2))
            pl.when(i + 1 < q2)(lambda: _wait(c_cp(i + 1 - q1)))
            now, ahead = jnp.maximum(i - q1, 0), jnp.minimum(i + 1, q2 - 1) - q1
            sweep(i, functools.partial(factor_units, cs_v.at[now]), lambda par: c_turns(ahead, 1 - par))

        _start(wo_cp(p) for p in range(nb, ng * ppg))

        @pl.loop(q2, n_blk)
        def _(i):
            p = i - q2
            pl.when(i == n_blk - 5)(lambda: w_start(0))
            pl.when(i == n_blk - 1)(lambda: w_start(1))
            wo_cp(p).wait()
            sweep(i, lambda par: wo_units(p))

    def output_dots(i, par):
        def halves(k):
            src, cols = states(i, par)[k * kc // P], pl.ds(k * kc % P, kc)
            return [src[pl.ds(4 * h, 4), :, cols].reshape(hb, kc) for h in range(2)]
        return product_dots(prod_v[par], halves, nc, lambda g, slot: cs_v[:, g, slot], nb)

    def output_units(i, par):
        total = functools.cache(lambda g, k: SSM.combine(lambda slot: prod_v[par][g, slot, pl.ds(8 * k, 8), :]))

        def unit(k, q):
            x = _halves(pltpu.bitcast(xp_v[i[0], k, :, lanes(q)], U32))
            ga_v[par][i[1], k, :, lanes(q)] = jnp.concatenate(
                [y[q % na] + v * coef_v[q, C_SKIP] for y, v in zip(total(q // na, k), x)], axis=0)
        return [(28 - 6 * j, functools.partial(unit, k, g * na + j))
                for g in range(nc) for k in range(TL // 2) for j in range(na)]

    def qkv_units(first, first_staged, par):
        src, dst = wst_v.at[:, :, pl.ds(first_staged, spp)], wqkv_v.at[pl.ds(first, spp)]

        def load(u, g, i):
            out = []
            for jp in range(g * n // 2, (g + 1) * n // 2):
                even, odd = (pltpu.bitcast(src[h, i, u, jp], U32) for h in range(2))
                words = (even & jnp.uint32(0xFFFF)) | (odd << 16), (even >> 16) | (odd & jnp.uint32(0xFFFF0000))
                out += zip(words, zip(_halves(even), _halves(odd)))
            return out

        def store(u, g, slot, v):
            dst[u, g, slot] = v
        return [v for at in list(itertools.product(range(spp), range(ng)))[par::2]
                for v in ATT.right_factor_units(functools.partial(load, *at), functools.partial(store, *at))]

    def s5_outputs_and_attention(bx_v, mem0_v, mem_v, pq_v):
        x_cp = [pltpu.make_async_copy(a, b, sems.at[SEM_BX]) for a, b in ((bx_hbm, bx_v), (mem0_hbm, mem0_v))]
        ya_cp = [pltpu.make_async_copy(ga_v[par].at[:, r // 2, pl.ds(r % 2 * 8, 8)],
                                       out_hbm.at[:, par, :, r, pl.ds(0, D)], sems.at[SEM_YA])
                 for par in range(2) for r in range(TL)]
        pair_rows = lambda k: (2 * seg * k // tb, pl.ds(2 * seg * k % tb // TL, 2 * seg // TL))

        def yb_start(k):
            blk, rows = pair_rows(k)
            pltpu.make_async_copy(gb_v.at[blk, rows], out_hbm.at[blk // 2, blk % 2, rows, :, pl.ds(D, Dm)],
                                  sems.at[SEM_YB]).start()

        w_wait(0)
        region(lambda i: _weave(output_dots(both(0), 0), scan_units(both(n_blk - 1), 1), qkv_units(i, 0, 0)))

        @pl.loop(1, n_blk)
        def _(i):
            for p in range(1, len(w_parts)):
                @pl.when(i == w_parts[p][0] // spp * 2)
                def _():
                    if p == 1:
                        w_start(2)
                        w_start(3)
                        _start(x_cp)
                    w_wait(p)
            cur, prev, at = both(i), both(jnp.maximum(i - 1, 0)), (i // 2 * spp, i // 2 * spp % ring)
            by_parity(i, lambda par: _weave(output_dots(cur, par), output_units(prev, 1 - par), qkv_units(*at, par)))

        _wait(x_cp)
        scale = float(Dh) ** -0.5
        key = lax.broadcasted_iota(jnp.int32, (L, L), 0)
        query = lax.broadcasted_iota(jnp.int32, (L, L), 1)
        mask = (query < M) | (query >= key)
        symmetric = [ATT.S(*p) for p in ATT.pairs]
        by_last = sorted(ATT.pairs, key=lambda p: p[::-1])
        qkv_order = list(range(n // 2)) + by_last[:2 * n] + list(range(n // 2, n)) + by_last[2 * n:]
        wo_order = list(range(n)) + ATT.pairs
        carried = [[s for s in ATT.half_slots(odd, wo_order, 1) if s not in symmetric] for odd in range(2)]
        qkv_weight = lambda w, g, slot: pltpu.bitcast(wqkv_v[pl.ds(w * slabs, slabs), g, slot].reshape(-1, LN), BF16)
        wo_weight = lambda slot, g0, g1: pltpu.bitcast(wo_v[pl.ds(g0 * ppg, (g1 - g0) * ppg), slot].reshape(-1, LN), BF16)

        def step_lhs(odd, slot, mem, own, other):
            rows = [ATT.single_factor(odd, mem, slot), own(slot)] + ([] if slot in symmetric else [other(slot)])
            return jnp.concatenate(rows, axis=0)

        def token_factors(s):
            rows = bx_v.at[pl.ds(pl.multiple_of(s * seg, seg), seg)]
            x1, x2 = (functools.cache(lambda i, r=r: rows[pl.ds(r, hs), lanes(i)].astype(F32)) for r in (0, hs))
            return ATT.left_factors(x1, functools.cache(lambda i: x2(i) - ATT.t[i] * x1(i)))

        def head_factors(odd, g0, g1):
            mem, x1, xi = (functools.cache(lambda i, r=r: o_v[odd][i, r, pl.ds(g0 * Dh, (g1 - g0) * Dh)])
                           for r in (pl.ds(0, M), pl.ds(M, hs), pl.ds(M + hs, hs)))
            return mem, ATT.left_factors(x1, xi)

        def store_segment(at, odd):
            for r in range(0, hs, 8):
                for j, y in enumerate(zip(*ATT.combine(lambda slot: po_v[odd][slot, pl.ds(r, 8), :]))):
                    for h in range(2):
                        gb_v.at[at][2 * odd + h, pl.ds(r, 8), lanes(j)] = y[h]

        def pair_of_steps(k):
            events = collections.defaultdict(list)
            clock = [0]

            def dot(lhs, rhs):
                while events and min(events) <= clock[0]:
                    for fn in events.pop(min(events)):
                        fn()
                clock[0] += rhs.shape[0] // LN
                return jnp.dot(lhs(), rhs, preferred_element_type=F32)

            def later(fn, g, delays):
                for delay, j in zip(delays, range(0, n, N_MXU), strict=True):
                    events[clock[0] + delay].append(functools.partial(fn, g, range(j, j + N_MXU)))

            def step(odd, own, ahead):
                store_segment(done, odd)
                mem = functools.cache(lambda i: mem_v[:, lanes(i)])
                lhs = functools.cache(lambda slot: step_lhs(odd, slot, mem, own, ahead))
                qkv, prob = {}, {}

                def project(g, w):
                    m = {}
                    for slot in ATT.half_slots(odd, qkv_order, N_MXU):
                        m[slot] = dot(lambda: lhs(slot), qkv_weight(w, g, slot))
                        if slot not in symmetric:
                            pq_v[odd][w, g, carried[odd].index(slot)] = m[slot][M + hs:]
                    parts = (ATT.single_combine(odd, lambda slot: m[slot][:M], qkv_order),
                             *ATT.combine(lambda slot: m[slot][M:M + hs] if slot in m
                                          else pq_v[1 - odd][w, g, carried[1 - odd].index(slot)], qkv_order))
                    for j, rows in enumerate(zip(*parts)):
                        qkv[g, j, w] = jnp.concatenate(rows, axis=0).astype(BF16 if w == 2 else F32)

                def softmax(g, heads):
                    for j in heads:
                        z = lax.dot_general(qkv.pop((g, j, 1)), qkv.pop((g, j, 0)), NT, preferred_element_type=F32)
                        z = jnp.where(mask, z * (scale * LOG2_E), -1e9 * LOG2_E)
                        e = jnp.exp2(z - jnp.max(z, axis=0, keepdims=True))
                        prob[g, j] = (e * pl.reciprocal(jnp.sum(e, axis=0, keepdims=True), full_range=False)).T

                def mix(g, heads):
                    for j in heads:
                        o = jnp.dot(prob.pop((g, j)), qkv.pop((g, j, 2)), preferred_element_type=F32)
                        o_v[odd][j, :, lanes(g)] = jnp.concatenate(
                            [o[:M + hs], o[M + hs:] - ATT.t[j] * o[M:M + hs]], axis=0)

                for g in range(ng):
                    project(g, 0)
                    project(g, 1)
                    later(softmax, g, (12, 36))
                    project(g, 2)
                    later(mix, g, (12, 16) if g < ng - 1 else (48, 72))

                heads = functools.cache(head_factors)
                part = lambda slot, g0, g1: dot(
                    lambda: step_lhs(odd, slot, *heads(odd, g0, g1), heads(1 - odd, g0, g1)[1]), wo_weight(slot, g0, g1))
                m = {slot: part(slot, 0, ng // 2) for slot in ATT.half_slots(odd, wo_order, 2)}
                for slot in m:
                    m[slot] = part(slot, ng // 2, ng) + m[slot]
                    po_v[odd][slot] = m[slot][M:M + hs]
                    if slot not in symmetric:
                        po_v[1 - odd][slot] = m[slot][M + hs:]
                for j, v in enumerate(ATT.single_combine(odd, lambda slot: m[slot][:M], wo_order)):
                    mem_v[:, lanes(j)] = v

            done = pair_rows(jnp.maximum(k - 1, 0))
            tokens = [token_factors(s) for s in (2 * k, 2 * k + 1, jnp.minimum(2 * k + 2, n_seg - 1))]
            step(0, *tokens[:2])
            step(1, *tokens[1:])
            assert not events
            pl.when(k > 0)(lambda: yb_start(k - 1))

        def before_first_step(_):
            first = token_factors(0)
            mem_v[...] = mem0_v[...].astype(F32)

            def dot(w, g, a):
                pq_v[1][w, g, a] = jnp.dot(first(carried[1][a]), qkv_weight(w, g, carried[1][a]),
                                           preferred_element_type=F32)
            _weave([(2, functools.partial(dot, *at))
                    for at in itertools.product(range(3), range(ng), range(len(carried[1])))],
                   output_units(both(n_blk - 1), 1))

        def after_last_step(_):
            last = head_factors(1, 0, ng)[1]
            for a, slot in enumerate(carried[0]):
                po_v[1][slot] = jnp.dot(last(slot), wo_weight(slot, 0, ng), preferred_element_type=F32)
                if a == n:
                    store_segment(pair_rows(n_seg // 2 - 1), 0)
            store_segment(pair_rows(n_seg // 2 - 1), 1)

        region(before_first_step)
        _start(ya_cp)
        pl.loop(0, n_seg // 2)(pair_of_steps)
        region(after_last_step)
        yb_start(n_seg // 2 - 1)
        _wait(ya_cp)
        pltpu.make_async_copy(gb_v, gb_v, sems.at[SEM_YB]).wait()

    pl.run_scoped(
        s5_states, pltpu.VMEM((4, P // LN, LN), BF16), pltpu.VMEM((ng * ppg, n, Dh // ppg, Dm), BF16),
        [pltpu.VMEM((nc, na, na, LN // 2, LN), U32)] * 2,
        pltpu.VMEM((nb, nc, SSM.slots, LN // 2, LN), U32))
    pl.run_scoped(
        s5_outputs_and_attention, pltpu.VMEM((S, Dm), BF16), pltpu.VMEM((M, Dm), BF16), pltpu.VMEM((M, Dm), F32),
        [pltpu.VMEM((3, ng, n + len(ATT.pairs), hs, Dh), F32)] * 2)


@functools.partial(jax.jit, static_argnames=("B_seg_len",))
def pallas_concat_heads__ssm_conv_s5__memory_aug_recurrent_mem_tr__prompt_kernel(
    A_x, A_Lambda_re, A_Lambda_im, A_B_re, A_B_im, A_C_re, A_C_im, A_log_dt, A_Dskip,
    B_x, B_mem0, B_Wq, B_Wk, B_Wv, B_Wo, B_seg_len,
):
    batch, S, D = A_x.shape
    P = A_B_re.shape[0]
    Dm, H, Dh = B_Wq.shape
    M = B_mem0.shape[1]
    seg = B_seg_len
    assert (batch, S, D, P, Dm, H, Dh, M, seg) == (1, 2048, 1024, 1024, 1024, 32, 128, 8, 32)
    n, ng, n_blk = ATT.n, H // ATT.n, S // (8 * TL)
    nb, nc = 2 * P // (SSM.n * LN), D // (SSM.n * LN)
    slabs = Dm // (n * 16)
    hbm = pl.BlockSpec(memory_space=pl.ANY)
    vec = lambda v: v.reshape(-1, LN)
    out = pl.pallas_call(
        functools.partial(_kernel, seg=seg),
        out_shape=jax.ShapeDtypeStruct((n_blk // 2, 2, 8, TL, D + Dm), F32),
        grid=(1,),
        in_specs=[hbm] * 15,
        out_specs=hbm,
        scratch_shapes=[
            pltpu.VMEM((n_blk, TL // 2, 16, D), BF16),
            pltpu.VMEM((nb, nc, SSM.slots, LN // 2, LN), U32),
            pltpu.VMEM((2, n, 2 * slabs + 2, H // 2, 16, Dh), BF16),
            pltpu.VMEM((3 * slabs, ng, ATT.slots, 8, Dh), U32),
            pltpu.VMEM((n_blk // 2, ATT.slots, ng * Dh // n_blk, LN), U32),
            [pltpu.VMEM((n_blk // 2, 8, TL, P), F32)] * 2,
            pltpu.VMEM((n_blk, 8, TL, P), F32),
            [pltpu.VMEM((nb, SSM.slots, 4 * TL, LN), F32)] * 2,
            pltpu.VMEM((P // LN, 9 + 2 * TL, 8, LN), F32),
            pltpu.VMEM((P // LN, 2, 8, LN), F32),
            [pltpu.VMEM((n, M + seg, ng * Dh), F32)] * 2,
            [pltpu.VMEM((ATT.slots, seg // 2, LN), F32)] * 2,
            pltpu.SemaphoreType.DMA((11 + 2 * nb + n_blk // 2,)),
        ],
        compiler_params=pltpu.CompilerParams(vmem_limit_bytes=126 * 2**20),
        name="fused_s5_rmt",
    )(A_x.reshape(n_blk, 8, TL, D), vec(A_Lambda_re), vec(A_Lambda_im),
      A_B_re.reshape(nb, n // 2, -1, D), A_B_im.reshape(nb, n // 2, -1, D),
      A_C_re.reshape(nc, n, -1, P), A_C_im.reshape(nc, n, -1, P),
      vec(A_log_dt), vec(A_Dskip), B_x.reshape(S, Dm), B_mem0.reshape(M, Dm),
      *(w.reshape(n, slabs, 16, H // 2, 2, Dh) for w in (B_Wq, B_Wk, B_Wv)),
      B_Wo.reshape(ng, n, Dh, Dm))
    return out.reshape(1, S, D + Dm)
```
